```python
import os as _os
_os.environ.setdefault("JAX_PLATFORMS", "cpu")
import jax
import jax.numpy as jnp

def _softmax(x, axis=-1):
    return jax.nn.softmax(x, axis=axis)
def _gelu(x):
    return jax.nn.gelu(x, approximate=True)
def _silu(x):
    return jax.nn.silu(x)
def _sigmoid(x):
    return jax.nn.sigmoid(x)
def _layernorm(x, axis=-1, eps=1e-5):
    m = jnp.mean(x, axis=axis, keepdims=True)
    v = jnp.var(x, axis=axis, keepdims=True)
    return (x - m) / jnp.sqrt(v + eps)
def _scatter_add(tgt, idx, src, axis=0):
    return tgt.at[idx].add(src)
def _segment_sum(src, seg, n):
    return jax.ops.segment_sum(src, seg, n)
class _Rng:
    def __init__(self, key):
        self._k = key
    def _next(self):
        self._k, sub = jax.random.split(self._k)
        return sub
    def normal(self, shape):
        return jax.random.normal(self._next(), shape, dtype=jnp.bfloat16)
    def randint(self, lo, hi, shape):
        return jax.random.randint(self._next(), shape, lo, hi, dtype=jnp.int32)
    def uniform(self, shape, lo=0.0, hi=1.0):
        return jax.random.uniform(self._next(), shape, jnp.bfloat16, lo, hi)
    def permutation(self, n):
        return jax.random.permutation(self._next(), n)


kernel_name = 'standalone__gqa_block_cached__near_ridge'

def setup_inputs():
    _rng = _Rng(jax.random.key(int.from_bytes(__import__("os").urandom(4), "little")))
    _w = (lambda a: (lambda t: t.astype(jnp.bfloat16) if jnp.issubdtype(t.dtype, jnp.floating) else t)(jnp.asarray(a)))
    B, Sq, D = 8, 144, 448
    Hq, Hkv, Sk, Dh = 16, 8, 2048, 256
    assert Hq % Hkv == 0, (Hq, Hkv)
    return {
        "x": _w((lambda *s: _rng.normal(s) * 0.8)(B, Sq, D)),
        "k_cache": _w((lambda *s: _rng.normal(s) * 0.8)(B, Hkv, Sk, Dh)),
        "v_cache": _w((lambda *s: _rng.normal(s) * 0.05)(B, Hkv, Sk, Dh)),
        "wq": _w((lambda *s: _rng.normal(s) * 0.8)(D, Hq * Dh) * (D ** -0.5)),
        "wo": _w((lambda *s: _rng.normal(s) * 0.05)(Hq * Dh, D) * ((Hq * Dh) ** -0.5)),
    }

def reference(x, k_cache, v_cache, wq, wo):
    B, Sq, D = x.shape
    Hq, Dh = 16, 256
    Hkv = k_cache.shape[1]
    rep = Hq // Hkv
    q = (lambda x, *d: x.transpose(*d))((x @ wq).reshape(B, Sq, Hq, Dh), 0, 2, 1, 3)
    k = jnp.repeat(k_cache, rep, axis=1)
    v = jnp.repeat(v_cache, rep, axis=1)
    scores = jnp.einsum("bhqd,bhkd->bhqk", q, k) * (Dh ** -0.5)
    p = _softmax(scores, axis=-1)
    o = jnp.einsum("bhqk,bhkd->bhqd", p, v)
    return (lambda x, *d: x.transpose(*d))(o, 0, 2, 1, 3).reshape(B, Sq, Hq * Dh) @ wo
```

```python
import jax
import jax.numpy as jnp
from jax import lax
import jax.experimental.pallas as pl
import jax.experimental.pallas.tpu as pltpu

LOG2E = 1.4426950408889634
NT = (((1,), (1,)), ((), ()))
F32 = jnp.float32
BF16 = jnp.bfloat16


def build(x, k_cache, v_cache, wq, wo, N=4, chunks=(512,) * 4, NSLOT=2, QG=2, OG=3, BA=4):
    B, Sq, D = x.shape
    _, Hkv, Sk, Dh = k_cache.shape
    Hq = wq.shape[1] // Dh
    rep = Hq // Hkv
    scale = (Dh ** -0.5) * LOG2E
    TOK = B * Sq
    x2 = x.reshape(TOK, D)
    woT = wo.T
    M = rep * Sq
    W = rep * Dh
    T = B * Hkv
    S = T // N
    HG = Hkv // N
    k3 = k_cache.reshape(S, N, Sk, Dh)
    v3 = v_cache.reshape(S, N, Sk, Dh)
    assert sum(chunks) == Sk
    offs = [sum(chunks[:c]) for c in range(len(chunks))]
    NQ = Hkv // QG
    NTILES = TOK // 128
    NO = NTILES // OG
    DP = (D + 127) // 128 * 128
    RA = BA * Sq

    def kernel(x_hbm, k_hbm, v_hbm, wq_hbm, wo_hbm, out_hbm,
               x_v, wq_v, wo_v, q_all, o_all, p_ref, kbuf, vbuf, y_v, ksem, vsem, wsem, qsem, osem):

        def kcopy(s, slot):
            return pltpu.make_async_copy(k_hbm.at[s], kbuf.at[slot], ksem.at[slot])

        def vcopy(s, slot):
            return pltpu.make_async_copy(v_hbm.at[s], vbuf.at[slot], vsem.at[slot])

        xa_copy = pltpu.make_async_copy(x_hbm.at[pl.ds(0, RA)], x_v.at[pl.ds(0, RA)], wsem.at[0])
        xb_copy = pltpu.make_async_copy(x_hbm.at[pl.ds(RA, TOK - RA)], x_v.at[pl.ds(RA, TOK - RA)], wsem.at[1])
        wocopy = pltpu.make_async_copy(wo_hbm, wo_v, wsem.at[2])

        def wqcopy(h):
            c0 = h * W if isinstance(h, int) else pl.multiple_of(h * W, 128)
            return pltpu.make_async_copy(wq_hbm.at[:, pl.ds(c0, W)], wq_v.at[h], qsem.at[h])

        def ocopy(i):
            r0 = i * OG * 128 if isinstance(i, int) else pl.multiple_of(i * OG * 128, 128)
            return pltpu.make_async_copy(y_v.at[pl.ds(r0, OG * 128)], out_hbm.at[pl.ds(r0, OG * 128)], osem.at[i])

        def qproj(h, b0, b1):
            q = jnp.dot(x_v[b0 * Sq:b1 * Sq, :], wq_v[h], preferred_element_type=F32) * scale
            q = q.astype(BF16)
            for b in range(b0, b1):
                for r in range(rep):
                    q_all[b, h, r * Sq:(r + 1) * Sq, :] = q[(b - b0) * Sq:(b - b0 + 1) * Sq, r * Dh:(r + 1) * Dh]

        wqcopy(0).start()
        xa_copy.start()
        xb_copy.start()
        wqcopy(0).wait()
        xa_copy.wait()
        for h in range(1, Hkv):
            wqcopy(h).start()
        for s in range(NSLOT):
            kcopy(s, s).start()
            vcopy(s, s).start()
        qproj(0, 0, BA)
        xb_copy.wait()
        for h in range(1, QG):
            wqcopy(h).wait()
        qproj(0, BA, B)
        for h in range(1, QG):
            qproj(h, 0, B)

        def qstep(i, carry):
            for u in range(QG):
                wqcopy(i * QG + u).wait()
            for u in range(QG):
                qproj(i * QG + u, 0, B)
            return carry

        lax.fori_loop(1, NQ, qstep, 0)

        def step(s, carry):
            slot = s % NSLOT
            kcopy(s, slot).wait()
            vcopy(s, slot).wait()
            b = s // HG
            hg = s % HG
            row0 = pl.multiple_of(b * Sq, 16)

            def qk(j):
                qq = q_all[b, hg * N + j]
                m = None
                l = None
                betas = []
                for c, (off, sz) in enumerate(zip(offs, chunks)):
                    sc = lax.dot_general(qq, kbuf[slot, j, off:off + sz, :], NT, preferred_element_type=F32)
                    mc = jnp.max(sc, axis=-1, keepdims=True)
                    m_new = mc if m is None else jnp.maximum(m, mc)
                    p = jnp.exp2(sc - m_new)
                    lc = p[:, 0:128]
                    for t in range(1, sz // 128):
                        lc = lc + p[:, t * 128:(t + 1) * 128]
                    if m is None:
                        l = lc
                        betas.append(None)
                    else:
                        beta = jnp.exp2(m - m_new)
                        l = l * beta + lc
                        betas.append(beta)
                    m = m_new
                    p_ref[j % 2, :, off:off + sz] = p.astype(BF16)
                lsum = jnp.sum(l, axis=-1, keepdims=True)
                r0 = pl.reciprocal(lsum, approx=True)
                linv = r0 * (2.0 - lsum * r0)
                return betas, linv

            def pv(j, st):
                betas, linv = st
                o = None
                for c, (off, sz) in enumerate(zip(offs, chunks)):
                    pc = p_ref[j % 2, :, off:off + sz]
                    oc = jnp.dot(pc, vbuf[slot, j, off:off + sz, :], preferred_element_type=F32)
                    o = oc if o is None else o * betas[c] + oc
                o = (o * linv).astype(BF16)
                for r in range(rep):
                    o_all[hg, pl.ds(row0, Sq), j * W + r * Dh: j * W + (r + 1) * Dh] = o[r * Sq:(r + 1) * Sq]

            for j in range(N):
                pv(j, qk(j))

            @pl.when(s + NSLOT < S)
            def _():
                kcopy(s + NSLOT, slot).start()
                vcopy(s + NSLOT, slot).start()

            @pl.when(s + NSLOT == S)
            def _():
                wocopy.start()
            return carry

        lax.fori_loop(0, S, step, 0)

        wocopy.wait()

        def ostep(i, carry):
            for u in range(OG):
                r0 = pl.multiple_of((i * OG + u) * 128, 128)
                yT = None
                for g in range(HG):
                    part = lax.dot_general(wo_v[:, g * N * W:(g + 1) * N * W], o_all[g, pl.ds(r0, 128), :], NT,
                                           preferred_element_type=F32)
                    yT = part if yT is None else yT + part
                yT = jnp.concatenate([yT, jnp.zeros((DP - D, 128), F32)], axis=0)
                y_v[pl.ds(r0, 128), :] = yT.T[:, :D].astype(BF16)
            ocopy(i).start()
            return carry

        lax.fori_loop(0, NO, ostep, 0)
        for i in range(NO):
            ocopy(i).wait()

    any_spec = pl.BlockSpec(memory_space=pl.ANY)
    out = pl.pallas_call(
        kernel,
        in_specs=[any_spec] * 5,
        out_specs=any_spec,
        out_shape=jax.ShapeDtypeStruct((TOK, D), x.dtype),
        scratch_shapes=[
            pltpu.VMEM((TOK, D), BF16),
            pltpu.VMEM((Hkv, D, W), BF16),
            pltpu.VMEM((D, Hq * Dh), BF16),
            pltpu.VMEM((B, Hkv, M, Dh), BF16),
            pltpu.VMEM((HG, TOK, N * W), BF16),
            pltpu.VMEM((2, M, Sk), BF16),
            pltpu.VMEM((NSLOT, N, Sk, Dh), BF16),
            pltpu.VMEM((NSLOT, N, Sk, Dh), BF16),
            pltpu.VMEM((TOK, D), BF16),
            pltpu.SemaphoreType.DMA((NSLOT,)),
            pltpu.SemaphoreType.DMA((NSLOT,)),
            pltpu.SemaphoreType.DMA((3,)),
            pltpu.SemaphoreType.DMA((Hkv,)),
            pltpu.SemaphoreType.DMA((NO,)),
        ],
        compiler_params=pltpu.CompilerParams(vmem_limit_bytes=110 * 1024 * 1024),
    )(x2, k3, v3, wq, woT)
    return out.reshape(B, Sq, D)

@jax.jit
def pallas_standalone__gqa_block_cached__near_ridge_kernel(x, k_cache, v_cache, wq, wo):
    return build(x, k_cache, v_cache, wq, wo)
```

```python
import jax
import jax.numpy as jnp
from jax import lax
import jax.experimental.pallas as pl
import jax.experimental.pallas.tpu as pltpu

LOG2E = 1.4426950408889634
NT = (((1,), (1,)), ((), ()))
F32 = jnp.float32
BF16 = jnp.bfloat16

N = 4
CHUNK = 256
NSLOT = 2
BA = 3
LANE = 128


@jax.jit
def pallas_standalone__gqa_block_cached__near_ridge_kernel(x, k_cache, v_cache, wq, wo):
    B, Sq, D = x.shape
    _, Hkv, Sk, Dh = k_cache.shape
    Hq = wq.shape[1] // Dh
    rep = Hq // Hkv
    scale = (Dh ** -0.5) * LOG2E
    TOK = B * Sq
    M = rep * Sq
    W = rep * Dh
    S = B * Hkv // N
    HG = Hkv // N
    NC = Sk // CHUNK
    NTILES = TOK // LANE
    RA = BA * Sq
    NP = N - 1
    pre = [g * N + j for g in range(HG) for j in range(NP)]
    horder = pre + [h for h in range(Hkv) if h not in pre]
    NPRE = len(pre)
    DF = D // LANE * LANE
    DR = D - DF
    assert Hkv % N == 0 and Sk % CHUNK == 0 and TOK % LANE == 0 and Sq % 16 == 0
    assert HG & (HG - 1) == 0 and (NTILES - 1) % HG == 0 and 0 < DR and DR % 16 == 0

    def kernel(x_hbm, k_hbm, v_hbm, wq_hbm, wo_hbm, out_hbm,
               x_v, wq_v, wo_v, q_all, o_all, p_ref, kbuf, vbuf, y_v, acc_v,
               ksem, vsem, wsem, qsem, osem):

        def kcopy(s, slot):
            return pltpu.make_async_copy(k_hbm.at[s], kbuf.at[slot], ksem.at[slot])

        def vcopy(s, slot):
            return pltpu.make_async_copy(v_hbm.at[s], vbuf.at[slot], vsem.at[slot])

        xa_copy = pltpu.make_async_copy(x_hbm.at[pl.ds(0, RA)], x_v.at[pl.ds(0, RA)], wsem.at[0])
        xb_copy = pltpu.make_async_copy(x_hbm.at[pl.ds(RA, TOK - RA)], x_v.at[pl.ds(RA, TOK - RA)],
                                        wsem.at[1])
        wocopies = [pltpu.make_async_copy(wo_hbm.at[:, pl.ds(g * N * W, N * W)], wo_v.at[g],
                                          wsem.at[2 + g]) for g in range(HG)]

        def wqcopy(i):
            return pltpu.make_async_copy(wq_hbm.at[:, pl.ds(horder[i] * W, W)], wq_v.at[i], qsem.at[i])

        def ocopy(t):
            r0 = t * LANE if isinstance(t, int) else pl.multiple_of(t * LANE, LANE)
            return pltpu.make_async_copy(y_v.at[pl.ds(r0, LANE)], out_hbm.at[pl.ds(r0, LANE)],
                                         osem.at[t])

        def project(xrows, i):
            q = jnp.dot(xrows, wq_v[i], preferred_element_type=F32) * scale
            return q.astype(BF16)

        def qproj(i, b0, b1):
            q = project(x_v[b0 * Sq:b1 * Sq, :], i)
            for b in range(b0, b1):
                for r in range(rep):
                    q_all[b, i, r * Sq:(r + 1) * Sq, :] = (
                        q[(b - b0) * Sq:(b - b0 + 1) * Sq, r * Dh:(r + 1) * Dh])

        wqcopy(0).start()
        xa_copy.start()
        xb_copy.start()
        wqcopy(0).wait()
        xa_copy.wait()
        for i in range(1, Hkv):
            wqcopy(i).start()
        for s in range(NSLOT):
            kcopy(s, s).start()
            vcopy(s, s).start()
        qproj(0, 0, BA)
        xb_copy.wait()
        qproj(0, BA, B)

        def qstep(i, carry):
            pltpu.make_async_copy(wq_v.at[i], wq_v.at[i], qsem.at[i]).wait()
            qproj(i, 0, B)
            return carry

        lax.fori_loop(1, NPRE, qstep, 0)
        for i in range(NPRE, Hkv):
            wqcopy(i).wait()

        def step(s, carry):
            slot = s & (NSLOT - 1)
            kcopy(s, slot).wait()
            vcopy(s, slot).wait()
            b = lax.shift_right_logical(s, HG.bit_length() - 1)
            hg = s & (HG - 1)
            row0 = pl.multiple_of(b * Sq, 16)

            ql = project(x_v[pl.ds(row0, Sq), :], NPRE + hg)
            ql = jnp.concatenate([ql[:, r * Dh:(r + 1) * Dh] for r in range(rep)], axis=0)

            def qk(j):
                qq = q_all[b, hg * NP + j] if j < NP else ql
                m = l = None
                betas = []
                for c in range(NC):
                    ks = slice(c * CHUNK, (c + 1) * CHUNK)
                    sc = lax.dot_general(qq, kbuf[slot, j, ks, :], NT, preferred_element_type=F32)
                    mc = jnp.max(sc, axis=-1, keepdims=True)
                    m_new = mc if m is None else jnp.maximum(m, mc)
                    p = jnp.exp2(sc - m_new)
                    lc = p[:, 0:LANE]
                    for t in range(1, CHUNK // LANE):
                        lc = lc + p[:, t * LANE:(t + 1) * LANE]
                    if m is None:
                        l = lc
                        betas.append(None)
                    else:
                        beta = jnp.exp2(m - m_new)
                        l = l * beta + lc
                        betas.append(beta)
                    m = m_new
                    p_ref[j % 2, :, ks] = p.astype(BF16)
                lsum = jnp.sum(l, axis=-1, keepdims=True)
                r0 = pl.reciprocal(lsum, approx=True)
                return betas, r0 * (2.0 - lsum * r0)

            def pv(j, betas, linv):
                o = None
                for c in range(NC):
                    ks = slice(c * CHUNK, (c + 1) * CHUNK)
                    oc = jnp.dot(p_ref[j % 2, :, ks], vbuf[slot, j, ks, :], preferred_element_type=F32)
                    o = oc if o is None else o * betas[c] + oc
                o = (o * linv).astype(BF16)
                for r in range(rep):
                    o_all[hg, pl.ds(row0, Sq), j * W + r * Dh:j * W + (r + 1) * Dh] = (
                        o[r * Sq:(r + 1) * Sq])

            for j in range(N):
                pv(j, *qk(j))

            @pl.when(s + NSLOT < S)
            def _():
                kcopy(s + NSLOT, slot).start()
                vcopy(s + NSLOT, slot).start()

            @pl.when(s + NSLOT == S)
            def _():
                for c in wocopies:
                    c.start()

            return carry

        lax.fori_loop(0, S, step, 0)

        for c in wocopies:
            c.wait()

        def opart(g, r0):
            lhs = jnp.concatenate([wo_v[g, DF:D, :], wo_v[g, 0:DF, :]], axis=0)
            return lax.dot_general(lhs, o_all[g, pl.ds(r0, LANE), :], NT, preferred_element_type=F32)

        def emit(yT, r0):
            yT = jnp.concatenate([yT[DR:], yT[:DR], jnp.zeros((LANE - DR, LANE), F32)], axis=0)
            y_v[pl.ds(r0, LANE), :] = yT.T[:, :D].astype(BF16)

        def ostep(i, carry):
            last = (NTILES - 1) * LANE
            yT = opart(i, last) + jnp.where(i > 0, acc_v[...], 0.0)
            acc_v[...] = yT
            emit(yT, last)

            @pl.when(i == HG - 1)
            def _():
                ocopy(NTILES - 1).start()

            per = (NTILES - 1) // HG
            for u in range(per):
                t = i * per + u
                r0 = pl.multiple_of(t * LANE, LANE)
                yT = opart(0, r0)
                for g in range(1, HG):
                    yT = yT + opart(g, r0)
                emit(yT, r0)
                ocopy(t).start()
            return carry

        lax.fori_loop(0, HG, ostep, 0)
        for t in range(NTILES):
            ocopy(t).wait()

    any_spec = pl.BlockSpec(memory_space=pl.ANY)
    out = pl.pallas_call(
        kernel,
        in_specs=[any_spec] * 5,
        out_specs=any_spec,
        out_shape=jax.ShapeDtypeStruct((TOK, D), x.dtype),
        scratch_shapes=[
            pltpu.VMEM((TOK, D), BF16),
            pltpu.VMEM((Hkv, D, W), BF16),
            pltpu.VMEM((HG, D, N * W), BF16),
            pltpu.VMEM((B, NPRE, M, Dh), BF16),
            pltpu.VMEM((HG, TOK, N * W), BF16),
            pltpu.VMEM((2, M, Sk), BF16),
            pltpu.VMEM((NSLOT, N, Sk, Dh), BF16),
            pltpu.VMEM((NSLOT, N, Sk, Dh), BF16),
            pltpu.VMEM((TOK, D), BF16),
            pltpu.VMEM((D, LANE), F32),
            pltpu.SemaphoreType.DMA((NSLOT,)),
            pltpu.SemaphoreType.DMA((NSLOT,)),
            pltpu.SemaphoreType.DMA((2 + HG,)),
            pltpu.SemaphoreType.DMA((Hkv,)),
            pltpu.SemaphoreType.DMA((NTILES,)),
        ],
        compiler_params=pltpu.CompilerParams(vmem_limit_bytes=100 * 1024 * 1024),
    )(x.reshape(TOK, D), k_cache.reshape(S, N, Sk, Dh), v_cache.reshape(S, N, Sk, Dh), wq, wo.T)
    return out.reshape(B, Sq, D)
```

```python
import jax
import jax.numpy as jnp
from jax import lax
import jax.experimental.pallas as pl
import jax.experimental.pallas.tpu as pltpu

NT = (((1,), (1,)), ((), ()))
F32 = jnp.float32
BF16 = jnp.bfloat16

N = 4
CHUNK = 256
NSLOT = 2
BA = 3
LANE = 128


@jax.jit
def pallas_standalone__gqa_block_cached__near_ridge_kernel(x, k_cache, v_cache, wq, wo):
    B, Sq, D = x.shape
    _, Hkv, Sk, Dh = k_cache.shape
    Hq = wq.shape[1] // Dh
    rep = Hq // Hkv
    scale = Dh ** -0.5
    TOK = B * Sq
    M = rep * Sq
    W = rep * Dh
    S = B * Hkv // N
    HG = Hkv // N
    NC = Sk // CHUNK
    NTILES = TOK // LANE
    RA = BA * Sq
    NP = N - 1
    pre = [g * N + j for g in range(HG) for j in range(NP)]
    horder = pre + [h for h in range(Hkv) if h not in pre]
    NPRE = len(pre)
    DF = D // LANE * LANE
    DR = D - DF
    assert Hkv % N == 0 and Sk % CHUNK == 0 and TOK % LANE == 0 and Sq % 16 == 0
    assert HG & (HG - 1) == 0 and (NTILES - 1) % HG == 0 and 0 < DR and DR % 16 == 0

    def kernel(x_hbm, k_hbm, v_hbm, wq_hbm, wo_hbm, out_hbm,
               x_v, wq_v, wo_v, q_all, o_all, p_ref, kbuf, vbuf, y_v, acc_v,
               ksem, vsem, wsem, qsem, osem):

        def kcopy(s, slot):
            return pltpu.make_async_copy(k_hbm.at[s], kbuf.at[slot], ksem.at[slot])

        def vcopy(s, slot):
            return pltpu.make_async_copy(v_hbm.at[s], vbuf.at[slot], vsem.at[slot])

        xa_copy = pltpu.make_async_copy(x_hbm.at[pl.ds(0, RA)], x_v.at[pl.ds(0, RA)], wsem.at[0])
        xb_copy = pltpu.make_async_copy(x_hbm.at[pl.ds(RA, TOK - RA)], x_v.at[pl.ds(RA, TOK - RA)],
                                        wsem.at[1])
        wocopies = [pltpu.make_async_copy(wo_hbm.at[:, pl.ds(g * N * W, N * W)], wo_v.at[g],
                                          wsem.at[2 + g]) for g in range(HG)]

        def wqcopy(i):
            return pltpu.make_async_copy(wq_hbm.at[:, pl.ds(horder[i] * W, W)], wq_v.at[i], qsem.at[i])

        def ocopy(t):
            r0 = t * LANE if isinstance(t, int) else pl.multiple_of(t * LANE, LANE)
            return pltpu.make_async_copy(y_v.at[pl.ds(r0, LANE)], out_hbm.at[pl.ds(r0, LANE)],
                                         osem.at[t])

        def project(xrows, i):
            q = jnp.dot(xrows, wq_v[i], preferred_element_type=F32) * scale
            return q.astype(BF16)

        def qproj(i, b0, b1):
            q = project(x_v[b0 * Sq:b1 * Sq, :], i)
            for b in range(b0, b1):
                for r in range(rep):
                    q_all[b, i, r * Sq:(r + 1) * Sq, :] = (
                        q[(b - b0) * Sq:(b - b0 + 1) * Sq, r * Dh:(r + 1) * Dh])

        wqcopy(0).start()
        xa_copy.start()
        xb_copy.start()
        wqcopy(0).wait()
        xa_copy.wait()
        for i in range(1, Hkv):
            wqcopy(i).start()
        for s in range(NSLOT):
            kcopy(s, s).start()
            vcopy(s, s).start()
        qproj(0, 0, BA)
        xb_copy.wait()
        qproj(0, BA, B)

        def qstep(i, carry):
            pltpu.make_async_copy(wq_v.at[i], wq_v.at[i], qsem.at[i]).wait()
            qproj(i, 0, B)
            return carry

        lax.fori_loop(1, NPRE, qstep, 0)
        for i in range(NPRE, Hkv):
            wqcopy(i).wait()

        def step(s, carry):
            slot = s & (NSLOT - 1)
            kcopy(s, slot).wait()
            vcopy(s, slot).wait()
            b = lax.shift_right_logical(s, HG.bit_length() - 1)
            hg = s & (HG - 1)
            row0 = pl.multiple_of(b * Sq, 16)

            ql = project(x_v[pl.ds(row0, Sq), :], NPRE + hg)
            ql = jnp.concatenate([ql[:, r * Dh:(r + 1) * Dh] for r in range(rep)], axis=0)

            def qk(j):
                qq = q_all[b, hg * NP + j] if j < NP else ql
                m = l = None
                betas = []
                for c in range(NC):
                    ks = slice(c * CHUNK, (c + 1) * CHUNK)
                    sc = lax.dot_general(qq, kbuf[slot, j, ks, :], NT, preferred_element_type=F32)
                    mc = jnp.max(sc, axis=-1, keepdims=True)
                    m_new = mc if m is None else jnp.maximum(m, mc)
                    p = jnp.exp(sc - m_new)
                    lc = p[:, 0:LANE]
                    for t in range(1, CHUNK // LANE):
                        lc = lc + p[:, t * LANE:(t + 1) * LANE]
                    if m is None:
                        l = lc
                        betas.append(None)
                    else:
                        beta = jnp.exp(m - m_new)
                        l = l * beta + lc
                        betas.append(beta)
                    m = m_new
                    p_ref[j % 2, :, ks] = p.astype(BF16)
                lsum = jnp.sum(l, axis=-1, keepdims=True)
                r0 = pl.reciprocal(lsum, approx=True)
                return betas, r0 * (2.0 - lsum * r0)

            def pv(j, betas, linv):
                o = None
                for c in range(NC):
                    ks = slice(c * CHUNK, (c + 1) * CHUNK)
                    oc = jnp.dot(p_ref[j % 2, :, ks], vbuf[slot, j, ks, :], preferred_element_type=F32)
                    o = oc if o is None else o * betas[c] + oc
                o = (o * linv).astype(BF16)
                for r in range(rep):
                    o_all[hg, pl.ds(row0, Sq), j * W + r * Dh:j * W + (r + 1) * Dh] = (
                        o[r * Sq:(r + 1) * Sq])

            for j in range(N):
                pv(j, *qk(j))

            @pl.when(s + NSLOT < S)
            def _():
                kcopy(s + NSLOT, slot).start()
                vcopy(s + NSLOT, slot).start()

            @pl.when(s + NSLOT == S)
            def _():
                for c in wocopies:
                    c.start()

            return carry

        lax.fori_loop(0, S, step, 0)

        for c in wocopies:
            c.wait()

        def opart(g, r0):
            lhs = jnp.concatenate([wo_v[g, DF:D, :], wo_v[g, 0:DF, :]], axis=0)
            return lax.dot_general(lhs, o_all[g, pl.ds(r0, LANE), :], NT, preferred_element_type=F32)

        def emit(yT, r0):
            yT = jnp.concatenate([yT[DR:], yT[:DR], jnp.zeros((LANE - DR, LANE), F32)], axis=0)
            y_v[pl.ds(r0, LANE), :] = yT.T[:, :D].astype(BF16)

        def ostep(i, carry):
            last = (NTILES - 1) * LANE
            yT = opart(i, last) + jnp.where(i > 0, acc_v[...], 0.0)
            acc_v[...] = yT
            emit(yT, last)

            @pl.when(i == HG - 1)
            def _():
                ocopy(NTILES - 1).start()

            per = (NTILES - 1) // HG
            for u in range(per):
                t = i * per + u
                r0 = pl.multiple_of(t * LANE, LANE)
                yT = opart(0, r0)
                for g in range(1, HG):
                    yT = yT + opart(g, r0)
                emit(yT, r0)
                ocopy(t).start()
            return carry

        lax.fori_loop(0, HG, ostep, 0)
        for t in range(NTILES):
            ocopy(t).wait()

    any_spec = pl.BlockSpec(memory_space=pl.ANY)
    out = pl.pallas_call(
        kernel,
        in_specs=[any_spec] * 5,
        out_specs=any_spec,
        out_shape=jax.ShapeDtypeStruct((TOK, D), x.dtype),
        scratch_shapes=[
            pltpu.VMEM((TOK, D), BF16),
            pltpu.VMEM((Hkv, D, W), BF16),
            pltpu.VMEM((HG, D, N * W), BF16),
            pltpu.VMEM((B, NPRE, M, Dh), BF16),
            pltpu.VMEM((HG, TOK, N * W), BF16),
            pltpu.VMEM((2, M, Sk), BF16),
            pltpu.VMEM((NSLOT, N, Sk, Dh), BF16),
            pltpu.VMEM((NSLOT, N, Sk, Dh), BF16),
            pltpu.VMEM((TOK, D), BF16),
            pltpu.VMEM((D, LANE), F32),
            pltpu.SemaphoreType.DMA((NSLOT,)),
            pltpu.SemaphoreType.DMA((NSLOT,)),
            pltpu.SemaphoreType.DMA((2 + HG,)),
            pltpu.SemaphoreType.DMA((Hkv,)),
            pltpu.SemaphoreType.DMA((NTILES,)),
        ],
        compiler_params=pltpu.CompilerParams(vmem_limit_bytes=100 * 1024 * 1024),
    )(x.reshape(TOK, D), k_cache.reshape(S, N, Sk, Dh), v_cache.reshape(S, N, Sk, Dh), wq, wo.T)
    return out.reshape(B, Sq, D)
```

```python
import jax
import jax.numpy as jnp
from jax import lax
import jax.experimental.pallas as pl
import jax.experimental.pallas.tpu as pltpu

NT = (((1,), (1,)), ((), ()))
F32 = jnp.float32
BF16 = jnp.bfloat16

N = 4
CHUNK = 256
NSLOT = 2
XSPLIT = (2, 3, 6)
QG = 2
LANE = 128


@jax.jit
def pallas_standalone__gqa_block_cached__near_ridge_kernel(x, k_cache, v_cache, wq, wo):
    B, Sq, D = x.shape
    _, Hkv, Sk, Dh = k_cache.shape
    Hq = wq.shape[1] // Dh
    rep = Hq // Hkv
    scale = Dh ** -0.5
    TOK = B * Sq
    M = rep * Sq
    W = rep * Dh
    S = B * Hkv // N
    HG = Hkv // N
    NC = Sk // CHUNK
    NTILES = TOK // LANE
    NP = N - 1
    pre = [g * N + j for g in range(HG) for j in range(NP)]
    horder = pre + [h for h in range(Hkv) if h not in pre]
    NPRE = len(pre)
    DF = D // LANE * LANE
    DR = D - DF
    xb = (0,) + XSPLIT + (B,)
    assert rep == 2 and Hkv % N == 0 and Sk % CHUNK == 0 and TOK % LANE == 0 and Sq % 16 == 0
    assert HG & (HG - 1) == 0 and (NTILES - 1) % HG == 0 and 0 < DR and DR % 16 == 0
    assert (NPRE - 2) % QG == 0 and XSPLIT[-1] < B

    def kernel(x_hbm, k_hbm, v_hbm, wq_hbm, wo_hbm, out_hbm,
               x_v, wq_v, wo_v, q_all, o_all, p_ref, kbuf, vbuf, y_v, acc_v,
               ksem, vsem, xsem, wsem, qsem, osem):

        def kcopy(s, slot):
            return pltpu.make_async_copy(k_hbm.at[s], kbuf.at[slot], ksem.at[slot])

        def vcopy(s, slot):
            return pltpu.make_async_copy(v_hbm.at[s], vbuf.at[slot], vsem.at[slot])

        def xcopy(i):
            rows = pl.ds(xb[i] * Sq, (xb[i + 1] - xb[i]) * Sq)
            return pltpu.make_async_copy(x_hbm.at[rows], x_v.at[rows], xsem.at[i])

        def wq0copy(r):
            return pltpu.make_async_copy(wq_hbm.at[:, pl.ds(horder[0] * W + r * Dh, Dh)],
                                         wq_v.at[0, :, pl.ds(r * Dh, Dh)], wsem.at[r])

        def wqcopy(i):
            return pltpu.make_async_copy(wq_hbm.at[:, pl.ds(horder[i] * W, W)], wq_v.at[i], qsem.at[i])

        def wocopy(g):
            return pltpu.make_async_copy(wo_hbm.at[:, pl.ds(g * N * W, N * W)], wo_v.at[g],
                                         wsem.at[rep + g])

        def ocopy(t):
            r0 = t * LANE if isinstance(t, int) else pl.multiple_of(t * LANE, LANE)
            return pltpu.make_async_copy(y_v.at[pl.ds(r0, LANE)], out_hbm.at[pl.ds(r0, LANE)],
                                         osem.at[t])

        def project(xrows, w):
            return (jnp.dot(xrows, w, preferred_element_type=F32) * scale).astype(BF16)

        def qproj(i, b0, b1, heads=range(rep)):
            c0 = heads[0] * Dh
            q = project(x_v[b0 * Sq:b1 * Sq, :], wq_v[i, :, c0:(heads[-1] + 1) * Dh])
            for b in range(b0, b1):
                for r in heads:
                    q_all[b, i, r * Sq:(r + 1) * Sq, :] = (
                        q[(b - b0) * Sq:(b - b0 + 1) * Sq, r * Dh - c0:(r + 1) * Dh - c0])

        wq0copy(0).start()
        xcopy(0).start()
        wq0copy(1).start()
        xcopy(1).start()
        wq0copy(0).wait()
        xcopy(2).start()
        xcopy(0).wait()
        qproj(0, xb[0], xb[1], heads=[0])

        wq0copy(1).wait()
        xcopy(3).start()
        xcopy(1).wait()
        wqcopy(1).start()
        qproj(0, xb[0], xb[1], heads=[1])
        qproj(0, xb[1], xb[2])

        xcopy(2).wait()
        qproj(0, xb[2], xb[3])

        xcopy(3).wait()
        wqcopy(1).wait()
        for i in range(2, Hkv):
            wqcopy(i).start()
        for s in range(NSLOT):
            kcopy(s, s).start()
            vcopy(s, s).start()
        qproj(0, xb[3], xb[4])
        qproj(1, 0, B)

        def qstep(it, carry):
            for u in range(QG):
                i = 2 + it * QG + u
                pltpu.make_async_copy(wq_v.at[i], wq_v.at[i], qsem.at[i]).wait()
            for u in range(QG):
                qproj(2 + it * QG + u, 0, B)
            return carry

        lax.fori_loop(0, (NPRE - 2) // QG, qstep, 0)
        for i in range(NPRE, Hkv):
            wqcopy(i).wait()

        def step(s, carry):
            slot = s & (NSLOT - 1)
            kcopy(s, slot).wait()
            vcopy(s, slot).wait()
            b = lax.shift_right_logical(s, HG.bit_length() - 1)
            hg = s & (HG - 1)
            row0 = pl.multiple_of(b * Sq, 16)

            ql = project(x_v[pl.ds(row0, Sq), :], wq_v[NPRE + hg])
            ql = jnp.concatenate([ql[:, r * Dh:(r + 1) * Dh] for r in range(rep)], axis=0)

            def qk(j):
                qq = q_all[b, hg * NP + j] if j < NP else ql
                m = l = None
                betas = []
                for c in range(NC):
                    ks = slice(c * CHUNK, (c + 1) * CHUNK)
                    sc = lax.dot_general(qq, kbuf[slot, j, ks, :], NT, preferred_element_type=F32)
                    mc = jnp.max(sc, axis=-1, keepdims=True)
                    m_new = mc if m is None else jnp.maximum(m, mc)
                    p = jnp.exp(sc - m_new)
                    lc = p[:, 0:LANE]
                    for t in range(1, CHUNK // LANE):
                        lc = lc + p[:, t * LANE:(t + 1) * LANE]
                    if m is None:
                        l = lc
                        betas.append(None)
                    else:
                        beta = jnp.exp(m - m_new)
                        l = l * beta + lc
                        betas.append(beta)
                    m = m_new
                    p_ref[j % 2, :, ks] = p.astype(BF16)
                lsum = jnp.sum(l, axis=-1, keepdims=True)
                r0 = pl.reciprocal(lsum, approx=True)
                return betas, r0 * (2.0 - lsum * r0)

            def pv(j, betas, linv):
                o = None
                for c in range(NC):
                    ks = slice(c * CHUNK, (c + 1) * CHUNK)
                    oc = jnp.dot(p_ref[j % 2, :, ks], vbuf[slot, j, ks, :], preferred_element_type=F32)
                    o = oc if o is None else o * betas[c] + oc
                o = (o * linv).astype(BF16)
                for r in range(rep):
                    o_all[hg, pl.ds(row0, Sq), j * W + r * Dh:j * W + (r + 1) * Dh] = (
                        o[r * Sq:(r + 1) * Sq])

            for j in range(N):
                pv(j, *qk(j))

            @pl.when(s + NSLOT < S)
            def _():
                kcopy(s + NSLOT, slot).start()
                vcopy(s + NSLOT, slot).start()

            @pl.when(s + NSLOT == S)
            def _():
                for g in range(HG):
                    wocopy(g).start()

            return carry

        lax.fori_loop(0, S, step, 0)

        for g in range(HG):
            wocopy(g).wait()

        def opart(g, r0):
            lhs = jnp.concatenate([wo_v[g, DF:D, :], wo_v[g, 0:DF, :]], axis=0)
            return lax.dot_general(lhs, o_all[g, pl.ds(r0, LANE), :], NT, preferred_element_type=F32)

        def emit(yT, r0):
            yT = jnp.concatenate([yT[DR:], yT[:DR], jnp.zeros((LANE - DR, LANE), F32)], axis=0)
            y_v[pl.ds(r0, LANE), :] = yT.T[:, :D].astype(BF16)

        def ostep(i, carry):
            last = (NTILES - 1) * LANE
            yT = opart(i, last) + jnp.where(i > 0, acc_v[...], 0.0)
            acc_v[...] = yT
            emit(yT, last)

            @pl.when(i == HG - 1)
            def _():
                ocopy(NTILES - 1).start()

            per = (NTILES - 1) // HG
            for u in range(per):
                t = i * per + u
                r0 = pl.multiple_of(t * LANE, LANE)
                yT = opart(0, r0)
                for g in range(1, HG):
                    yT = yT + opart(g, r0)
                emit(yT, r0)
                ocopy(t).start()
            return carry

        lax.fori_loop(0, HG, ostep, 0)
        for t in range(NTILES):
            ocopy(t).wait()

    any_spec = pl.BlockSpec(memory_space=pl.ANY)
    out = pl.pallas_call(
        kernel,
        in_specs=[any_spec] * 5,
        out_specs=any_spec,
        out_shape=jax.ShapeDtypeStruct((TOK, D), x.dtype),
        scratch_shapes=[
            pltpu.VMEM((TOK, D), BF16),
            pltpu.VMEM((Hkv, D, W), BF16),
            pltpu.VMEM((HG, D, N * W), BF16),
            pltpu.VMEM((B, NPRE, M, Dh), BF16),
            pltpu.VMEM((HG, TOK, N * W), BF16),
            pltpu.VMEM((2, M, Sk), BF16),
            pltpu.VMEM((NSLOT, N, Sk, Dh), BF16),
            pltpu.VMEM((NSLOT, N, Sk, Dh), BF16),
            pltpu.VMEM((TOK, D), BF16),
            pltpu.VMEM((D, LANE), F32),
            pltpu.SemaphoreType.DMA((NSLOT,)),
            pltpu.SemaphoreType.DMA((NSLOT,)),
            pltpu.SemaphoreType.DMA((len(xb) - 1,)),
            pltpu.SemaphoreType.DMA((rep + HG,)),
            pltpu.SemaphoreType.DMA((Hkv,)),
            pltpu.SemaphoreType.DMA((NTILES,)),
        ],
        compiler_params=pltpu.CompilerParams(vmem_limit_bytes=100 * 1024 * 1024),
    )(x.reshape(TOK, D), k_cache.reshape(S, N, Sk, Dh), v_cache.reshape(S, N, Sk, Dh), wq, wo.T)
    return out.reshape(B, Sq, D)
```
